```python
import os as _os
_os.environ.setdefault("JAX_PLATFORMS", "cpu")
import jax
import jax.numpy as jnp

def _softmax(x, axis=-1):
    return jax.nn.softmax(x, axis=axis)
def _gelu(x):
    return jax.nn.gelu(x, approximate=True)
def _silu(x):
    return jax.nn.silu(x)
def _sigmoid(x):
    return jax.nn.sigmoid(x)
def _layernorm(x, axis=-1, eps=1e-5):
    m = jnp.mean(x, axis=axis, keepdims=True)
    v = jnp.var(x, axis=axis, keepdims=True)
    return (x - m) / jnp.sqrt(v + eps)
def _scatter_add(tgt, idx, src, axis=0):
    return tgt.at[idx].add(src)
def _segment_sum(src, seg, n):
    return jax.ops.segment_sum(src, seg, n)
class _Rng:
    def __init__(self, key):
        self._k = key
    def _next(self):
        self._k, sub = jax.random.split(self._k)
        return sub
    def normal(self, shape):
        return jax.random.normal(self._next(), shape, dtype=jnp.bfloat16)
    def randint(self, lo, hi, shape):
        return jax.random.randint(self._next(), shape, lo, hi, dtype=jnp.int32)
    def uniform(self, shape, lo=0.0, hi=1.0):
        return jax.random.uniform(self._next(), shape, jnp.bfloat16, lo, hi)
    def permutation(self, n):
        return jax.random.permutation(self._next(), n)


kernel_name = 'standalone__gqa_block_cached__near_ridge'

def setup_inputs():
    _rng = _Rng(jax.random.key(int.from_bytes(__import__("os").urandom(4), "little")))
    _w = (lambda a: (lambda t: t.astype(jnp.bfloat16) if jnp.issubdtype(t.dtype, jnp.floating) else t)(jnp.asarray(a)))
    B, Sq, D = 32, 112, 448
    Hq, Hkv, Sk, Dh = 16, 8, 512, 256
    assert Hq % Hkv == 0, (Hq, Hkv)
    return {
        "x": _w((lambda *s: _rng.normal(s) * 0.8)(B, Sq, D)),
        "k_cache": _w((lambda *s: _rng.normal(s) * 0.8)(B, Hkv, Sk, Dh)),
        "v_cache": _w((lambda *s: _rng.normal(s) * 0.05)(B, Hkv, Sk, Dh)),
        "wq": _w((lambda *s: _rng.normal(s) * 0.8)(D, Hq * Dh) * (D ** -0.5)),
        "wo": _w((lambda *s: _rng.normal(s) * 0.05)(Hq * Dh, D) * ((Hq * Dh) ** -0.5)),
    }

def reference(x, k_cache, v_cache, wq, wo):
    B, Sq, D = x.shape
    Hq, Dh = 16, 256
    Hkv = k_cache.shape[1]
    rep = Hq // Hkv
    q = (lambda x, *d: x.transpose(*d))((x @ wq).reshape(B, Sq, Hq, Dh), 0, 2, 1, 3)
    k = jnp.repeat(k_cache, rep, axis=1)
    v = jnp.repeat(v_cache, rep, axis=1)
    scores = jnp.einsum("bhqd,bhkd->bhqk", q, k) * (Dh ** -0.5)
    p = _softmax(scores, axis=-1)
    o = jnp.einsum("bhqk,bhkd->bhqd", p, v)
    return (lambda x, *d: x.transpose(*d))(o, 0, 2, 1, 3).reshape(B, Sq, Hq * Dh) @ wo
```

```python
import functools
import jax
import jax.numpy as jnp
import jax.experimental.pallas as pl
import jax.experimental.pallas.tpu as pltpu

HQ = 16
DH = 256
GB = 8
HP = 2
LOG2E = 1.4426950408889634
NT = (((1,), (1,)), ((), ()))


def _kernel(x_hbm, k_hbm, v_hbm, wq_hbm, wot_hbm, o_hbm,
            x_v, wq_v, wo_v, k_v, v_v, q_s, acc, out_v,
            x_sem, wq_sem, wo_sem, k_sem, v_sem, o_sem,
            *, sq, hkv, rep, ngroups):
    m = GB * sq
    cw = rep * DH
    npair = hkv // HP
    nit = ngroups * npair
    pshift = npair.bit_length() - 1
    assert npair == 1 << pshift
    assert hkv == GB
    ntile = m // 128

    def gp(it):
        return jax.lax.shift_right_logical(it, jnp.int32(pshift)), it & (npair - 1)

    def x_copy(g):
        return pltpu.make_async_copy(x_hbm.at[pl.ds(g * m, m), :], x_v.at[g & 1], x_sem.at[g & 1])

    def wq_copy(h):
        return pltpu.make_async_copy(wq_hbm.at[:, pl.ds(h * cw, cw)], wq_v.at[h], wq_sem.at[h])

    def wo_copy(p):
        return pltpu.make_async_copy(wot_hbm.at[:, pl.ds(p * HP * cw, HP * cw)], wo_v.at[p], wo_sem.at[p])

    def kv_copy(src, dst, sem, it):
        g, p = gp(it)
        slot = it & 1
        return pltpu.make_async_copy(src.at[pl.ds(g * GB, GB), pl.ds(p * HP, HP)], dst.at[slot], sem.at[slot])

    k_copy = functools.partial(kv_copy, k_hbm, k_v, k_sem)
    v_copy = functools.partial(kv_copy, v_hbm, v_v, v_sem)

    def kv0_piece(src, dst, sem, b):
        return pltpu.make_async_copy(src.at[b, pl.ds(0, HP)], dst.at[0, b], sem.at[0])

    def out_copy(g):
        return pltpu.make_async_copy(out_v, o_hbm.at[pl.ds(g * m, m), :], o_sem.at[0])

    def qpiece(g, h, r):
        q = jnp.dot(x_v[g & 1], wq_v[h, :, r * DH:(r + 1) * DH], preferred_element_type=jnp.float32)
        q = (q * (DH ** -0.5 * LOG2E)).astype(jnp.bfloat16)
        for b in range(GB):
            q_s[g & 1, h, b, r * sq:(r + 1) * sq, :] = q[b * sq:(b + 1) * sq]

    def main_compute(it, with_q):
        g, p = gp(it)
        slot = it & 1
        gs = g & 1

        def qk(hh, b):
            return jax.lax.dot_general(q_s[gs, p * HP + hh, b], k_v[slot, b, hh], NT,
                                       preferred_element_type=jnp.float32)

        def pv(s, hh, b):
            mx = jnp.max(s, axis=-1, keepdims=True)
            e = jnp.exp2(s - mx)
            l = jnp.sum(e, axis=-1, keepdims=True)
            o = jnp.dot(e.astype(jnp.bfloat16), v_v[slot, b, hh], preferred_element_type=jnp.float32)
            o = (o * (1.0 / l)).astype(jnp.bfloat16)
            return jnp.concatenate([o[r * sq:(r + 1) * sq] for r in range(rep)], axis=1)

        rows = [[] for _ in range(HP)]

        def otile(hh, j):
            a = jnp.concatenate(rows[hh], axis=0)[j * 128:(j + 1) * 128]
            acc[:, j * 128:(j + 1) * 128] += jax.lax.dot_general(
                wo_v[p, :, hh * cw:(hh + 1) * cw], a, NT, preferred_element_type=jnp.float32)

        qpieces = [(hh, r) for hh in range(HP) for r in range(rep)] if with_q else []

        def emit_q():
            if qpieces:
                hh, r = qpieces.pop(0)
                qpiece(g + 1, p * HP + hh, r)

        seq = [(hh, b) for hh in range(HP) for b in range(GB)]
        n = len(seq)
        pending = [(hh, j) for hh in range(HP) for j in range(ntile)]
        s_next = qk(*seq[0])
        emit_q()
        for i, (hh, b) in enumerate(seq):
            s = s_next
            if i + 1 < n:
                s_next = qk(*seq[i + 1])
            if i == n - 1:
                emit_q()
            rows[hh].append(pv(s, hh, b))
            while pending:
                th, j = pending[0]
                last_b = ((j + 1) * 128 - 1) // sq
                if th * GB + last_b < i:
                    otile(th, j)
                    pending.pop(0)
                else:
                    break
            if i == GB - 1 or i == GB + 3 or (HP == 1 and i == 3):
                emit_q()
        while pending:
            if len(pending) == 1:
                emit_q()
            otile(*pending.pop(0))
        while qpieces:
            emit_q()

    def finalize(g):
        out_v[...] = acc[...].T.astype(out_v.dtype)
        acc[...] = jnp.zeros(acc.shape, acc.dtype)
        out_copy(g).start()

    def body(it, c, with_q):
        g, p = gp(it)

        @pl.when(it + 1 < nit)
        def _():
            k_copy(it + 1).start()
            v_copy(it + 1).start()

        @pl.when(it + 1 < npair)
        def _():
            wo_copy(it + 1).start()

        @pl.when(jnp.logical_and(p == 1, g + 2 < ngroups))
        def _():
            x_copy(g + 2).start()

        @pl.when(jnp.logical_and(p == 0, g + 1 < ngroups))
        def _():
            x_copy(g + 1).wait()

        @pl.when(it < npair)
        def _():
            wo_copy(it).wait()

        k_copy(it).wait()
        v_copy(it).wait()

        main_compute(it, with_q)

        @pl.when(p == npair - 1)
        def _():
            @pl.when(g > 0)
            def _():
                out_copy(g - 1).wait()
            finalize(g)
        return c

    x_copy(0).start()
    wq_copy(0).start()
    acc[...] = jnp.zeros(acc.shape, acc.dtype)

    def pro_body(h, c):
        @pl.when(h + 1 < hkv)
        def _():
            wq_copy(h + 1).start()

        kv0_piece(k_hbm, k_v, k_sem, h).start()
        kv0_piece(v_hbm, v_v, v_sem, h).start()

        @pl.when(h == 0)
        def _():
            x_copy(0).wait()

        @pl.when(h == 4)
        def _():
            wo_copy(0).start()

        @pl.when(h == 6)
        def _():
            if ngroups > 1:
                x_copy(1).start()

        wq_copy(h).wait()
        for r in range(rep):
            qpiece(0, h, r)
        return c

    jax.lax.fori_loop(0, hkv, pro_body, 0)
    jax.lax.fori_loop(0, nit - npair, functools.partial(body, with_q=True), 0)
    jax.lax.fori_loop(nit - npair, nit, functools.partial(body, with_q=False), 0)
    out_copy(ngroups - 1).wait()


@jax.jit
def pallas_standalone__gqa_block_cached__near_ridge_kernel(x, k_cache, v_cache, wq, wo):
    B, Sq, D = x.shape
    _, Hkv, Sk, Dh = k_cache.shape
    rep = HQ // Hkv
    ngroups = B // GB
    m = GB * Sq
    cw = rep * Dh
    bf = jnp.bfloat16
    kern = functools.partial(_kernel, sq=Sq, hkv=Hkv, rep=rep, ngroups=ngroups)
    hbm = pl.BlockSpec(memory_space=pltpu.HBM)
    out = pl.pallas_call(
        kern,
        in_specs=[hbm] * 5,
        out_specs=hbm,
        out_shape=jax.ShapeDtypeStruct((B * Sq, D), x.dtype),
        scratch_shapes=[
            pltpu.VMEM((2, m, D), bf),
            pltpu.VMEM((Hkv, D, cw), bf),
            pltpu.VMEM((Hkv // HP, D, HP * cw), bf),
            pltpu.VMEM((2, GB, HP, Sk, Dh), bf),
            pltpu.VMEM((2, GB, HP, Sk, Dh), bf),
            pltpu.VMEM((2, Hkv, GB, rep * Sq, Dh), bf),
            pltpu.VMEM((D, m), jnp.float32),
            pltpu.VMEM((m, D), bf),
            pltpu.SemaphoreType.DMA((2,)),
            pltpu.SemaphoreType.DMA((Hkv,)),
            pltpu.SemaphoreType.DMA((Hkv // HP,)),
            pltpu.SemaphoreType.DMA((2,)),
            pltpu.SemaphoreType.DMA((2,)),
            pltpu.SemaphoreType.DMA((1,)),
        ],
        compiler_params=pltpu.CompilerParams(
            vmem_limit_bytes=100 * 1024 * 1024,
            disable_bounds_checks=True,
        ),
    )(x.reshape(B * Sq, D), k_cache, v_cache, wq, wo.T)
    return out.reshape(B, Sq, D)
```

```python
import functools
import jax
import jax.numpy as jnp
import jax.experimental.pallas as pl
import jax.experimental.pallas.tpu as pltpu

HQ = 16
DH = 256
GB = 8
HP = 2
LOG2E = 1.4426950408889634
DEPTH = 2
ODELAY = 1
ORDER = 'QSPO'
SAHEAD = 0
PRENORM = False
NT = (((1,), (1,)), ((), ()))


def _kernel(x_hbm, k_hbm, v_hbm, wq_hbm, wot_hbm, o_hbm,
            x_v, wq_v, wo_v, kv_v, q_s, acc, out_v,
            x_sem, wq_sem, wq0_sem, wo_sem, kv_sem, o_sem,
            *, sq, hkv, rep, ngroups):
    m = GB * sq
    cw = rep * DH
    npair = hkv // HP
    nit = ngroups * npair
    pshift = npair.bit_length() - 1
    assert npair == 1 << pshift
    assert hkv == GB
    ntile = m // 128

    def gp(it):
        return jax.lax.shift_right_logical(it, jnp.int32(pshift)), it & (npair - 1)

    def x_copy(g):
        return pltpu.make_async_copy(x_hbm.at[pl.ds(g * m, m), :], x_v, x_sem.at[0])

    def x0_half_copy(half):
        rows = pl.ds(half * (m // 2), m // 2)
        return pltpu.make_async_copy(x_hbm.at[rows, :], x_v.at[rows, :], x_sem.at[half])

    def wq_copy(h):
        return pltpu.make_async_copy(wq_hbm.at[:, pl.ds(h * cw, cw)], wq_v.at[h], wq_sem.at[h])

    def wq0_part_copy(r):
        cols = pl.ds(r * DH, DH)
        return pltpu.make_async_copy(wq_hbm.at[:, cols], wq_v.at[0, :, cols], wq0_sem.at[r])

    def wo_copy(p):
        return pltpu.make_async_copy(wot_hbm.at[:, pl.ds(p * HP * cw, HP * cw)], wo_v.at[p], wo_sem.at[p])

    def kv_copy(src, which, it):
        g, p = gp(it)
        slot = it & 1
        return pltpu.make_async_copy(src.at[pl.ds(g * GB, GB), pl.ds(p * HP, HP)], kv_v.at[slot, which],
                                     kv_sem.at[slot])

    k_copy = functools.partial(kv_copy, k_hbm, 0)
    v_copy = functools.partial(kv_copy, v_hbm, 1)

    def kv_wait(it):
        slot = it & 1
        pltpu.make_async_copy(kv_v.at[slot], kv_v.at[slot], kv_sem.at[slot]).wait()

    def kv0_piece(src, which, b):
        return pltpu.make_async_copy(src.at[b, pl.ds(0, HP)], kv_v.at[0, which, b], kv_sem.at[0])

    def out_copy(g):
        return pltpu.make_async_copy(out_v, o_hbm.at[pl.ds(g * m, m), :], o_sem.at[0])

    def out_tile_copy(g, j):
        return pltpu.make_async_copy(out_v.at[pl.ds(j * 128, 128), :],
                                     o_hbm.at[pl.ds(g * m + j * 128, 128), :], o_sem.at[0])

    def qpiece(h, r, b0=0, b1=GB):
        q = jnp.dot(x_v[b0 * sq:b1 * sq, :], wq_v[h, :, r * DH:(r + 1) * DH],
                    preferred_element_type=jnp.float32)
        q = (q * (DH ** -0.5 * LOG2E)).astype(jnp.bfloat16)
        for b in range(b0, b1):
            q_s[h, b, r * sq:(r + 1) * sq, :] = q[(b - b0) * sq:(b - b0 + 1) * sq]

    def attention(it):
        g, p = gp(it)
        slot = it & 1

        def qk(hh, b):
            return jax.lax.dot_general(q_s[p * HP + hh, b], kv_v[slot, 0, b, hh], NT,
                                       preferred_element_type=jnp.float32)

        def soft(s):
            mx = jnp.max(s, axis=-1, keepdims=True)
            e = jnp.exp2(s - mx)
            l = jnp.sum(e, axis=-1, keepdims=True)
            if PRENORM:
                e = e * (1.0 / l)
            return e.astype(jnp.bfloat16), l

        def pv(el, hh, b):
            e, l = el
            o = jnp.dot(e, kv_v[slot, 1, b, hh], preferred_element_type=jnp.float32)
            if not PRENORM:
                o = o * (1.0 / l)
            o = o.astype(jnp.bfloat16)
            return jnp.concatenate([o[r * sq:(r + 1) * sq] for r in range(rep)], axis=1)

        rows = [[] for _ in range(HP)]

        def otile(hh, j):
            a = jnp.concatenate(rows[hh], axis=0)[j * 128:(j + 1) * 128]
            part = jax.lax.dot_general(
                wo_v[p, :, hh * cw:(hh + 1) * cw], a, NT, preferred_element_type=jnp.float32)
            old = acc[:, j * 128:(j + 1) * 128]
            if hh == 0:
                old = jnp.where(p == 0, 0.0, old)
            acc[:, j * 128:(j + 1) * 128] = old + part

        seq = [(hh, b) for hh in range(HP) for b in range(GB)]
        n = len(seq)
        pending = [(hh, j) for hh in range(HP) for j in range(ntile)]
        svals = [qk(*seq[i]) for i in range(DEPTH)]
        evals = [soft(svals[i]) for i in range(SAHEAD)]
        for i, (hh, b) in enumerate(seq):
            done = i
            for op in ORDER:
                if op == 'Q':
                    if i + DEPTH < n:
                        svals.append(qk(*seq[i + DEPTH]))
                elif op == 'S':
                    if i + SAHEAD < n:
                        evals.append(soft(svals[i + SAHEAD]))
                elif op == 'P':
                    rows[hh].append(pv(evals[i], hh, b))
                    done = i + 1
                else:
                    while pending:
                        th, j = pending[0]
                        last_b = ((j + 1) * 128 - 1) // sq
                        if th * GB + last_b + ODELAY <= i and th * GB + last_b < done:
                            otile(th, j)
                            pending.pop(0)
                        else:
                            break
        while pending:
            otile(*pending.pop(0))

    def body(it, c):
        g, p = gp(it)

        @pl.when(it < npair)
        def _():
            wo_copy(it).wait()

        kv_wait(it)

        @pl.when(it + 1 < nit)
        def _():
            k_copy(it + 1).start()
            v_copy(it + 1).start()

        @pl.when(it + 1 < npair)
        def _():
            wo_copy(it + 1).start()

        @pl.when(jnp.logical_and(p == 1, g + 1 < ngroups))
        def _():
            x_copy(g + 1).start()

        attention(it)

        @pl.when(jnp.logical_and(p == npair - 1, g + 1 < ngroups))
        def _():
            x_copy(g + 1).wait()

            @pl.when(g > 0)
            def _():
                out_copy(g - 1).wait()
            out_v[...] = acc[...].T.astype(out_v.dtype)
            out_copy(g).start()
            for h in range(hkv):
                for r in range(rep):
                    qpiece(h, r)
        return c

    x0_half_copy(0).start()
    wq0_part_copy(0).start()
    x0_half_copy(1).start()
    for r in range(1, rep):
        wq0_part_copy(r).start()
    x0_half_copy(0).wait()
    wq0_part_copy(0).wait()
    wq_copy(1).start()
    qpiece(0, 0, 0, GB // 2)
    x0_half_copy(1).wait()
    for b in range(2):
        kv0_piece(k_hbm, 0, b).start()
        kv0_piece(v_hbm, 1, b).start()
    qpiece(0, 0, GB // 2, GB)
    for r in range(1, rep):
        wq0_part_copy(r).wait()
        qpiece(0, r)

    def pro_body(h, c):
        wq_copy(h).wait()

        @pl.when(h + 1 < hkv)
        def _():
            wq_copy(h + 1).start()
            kv0_piece(k_hbm, 0, h + 1).start()
            kv0_piece(v_hbm, 1, h + 1).start()

        @pl.when(h == 4)
        def _():
            wo_copy(0).start()

        for r in range(rep):
            qpiece(h, r)
        return c

    jax.lax.fori_loop(1, hkv, pro_body, 0)
    jax.lax.fori_loop(0, nit, body, 0)

    gl = ngroups - 1
    if ngroups > 1:
        out_copy(gl - 1).wait()
    for j in range(ntile):
        out_v[j * 128:(j + 1) * 128, :] = acc[:, j * 128:(j + 1) * 128].T.astype(out_v.dtype)
        out_tile_copy(gl, j).start()
    out_copy(gl).wait()


@jax.jit
def pallas_standalone__gqa_block_cached__near_ridge_kernel(x, k_cache, v_cache, wq, wo):
    B, Sq, D = x.shape
    _, Hkv, Sk, Dh = k_cache.shape
    rep = HQ // Hkv
    ngroups = B // GB
    m = GB * Sq
    cw = rep * Dh
    bf = jnp.bfloat16
    kern = functools.partial(_kernel, sq=Sq, hkv=Hkv, rep=rep, ngroups=ngroups)
    hbm = pl.BlockSpec(memory_space=pltpu.HBM)
    out = pl.pallas_call(
        kern,
        in_specs=[hbm] * 5,
        out_specs=hbm,
        out_shape=jax.ShapeDtypeStruct((B * Sq, D), x.dtype),
        scratch_shapes=[
            pltpu.VMEM((m, D), bf),
            pltpu.VMEM((Hkv, D, cw), bf),
            pltpu.VMEM((Hkv // HP, D, HP * cw), bf),
            pltpu.VMEM((2, 2, GB, HP, Sk, Dh), bf),
            pltpu.VMEM((Hkv, GB, rep * Sq, Dh), bf),
            pltpu.VMEM((D, m), jnp.float32),
            pltpu.VMEM((m, D), bf),
            pltpu.SemaphoreType.DMA((2,)),
            pltpu.SemaphoreType.DMA((Hkv,)),
            pltpu.SemaphoreType.DMA((rep,)),
            pltpu.SemaphoreType.DMA((Hkv // HP,)),
            pltpu.SemaphoreType.DMA((2,)),
            pltpu.SemaphoreType.DMA((1,)),
        ],
        compiler_params=pltpu.CompilerParams(
            vmem_limit_bytes=126 * 1024 * 1024,
            disable_bounds_checks=True,
        ),
    )(x.reshape(B * Sq, D), k_cache, v_cache, wq, wo.T)
    return out.reshape(B, Sq, D)
```

```python
import functools
import jax
import jax.numpy as jnp
import jax.experimental.pallas as pl
import jax.experimental.pallas.tpu as pltpu

HQ = 16
DH = 256
GB = 8
HP = 2
DEPTH = 2
LOG2E = 1.4426950408889634
NT = (((1,), (1,)), ((), ()))


def _kernel(x_hbm, k_hbm, v_hbm, wq_hbm, wot_hbm, o_hbm,
            x_v, wq_v, wo_v, kv_v, q_s, acc, out_v,
            x_sem, wq_sem, wq0_sem, wo_sem, kv_sem, o_sem,
            *, sq, hkv, rep, ngroups):
    m = GB * sq
    cw = rep * DH
    npair = hkv // HP
    nit = ngroups * npair
    pshift = npair.bit_length() - 1
    assert npair == 1 << pshift
    assert hkv == 8 and GB == 8
    ntile = m // 128

    def gp(it):
        return jax.lax.shift_right_logical(it, jnp.int32(pshift)), it & (npair - 1)

    def x_copy(g):
        return pltpu.make_async_copy(x_hbm.at[pl.ds(g * m, m), :], x_v, x_sem.at[0])

    def x0_half_copy(half):
        rows = pl.ds(half * (m // 2), m // 2)
        return pltpu.make_async_copy(x_hbm.at[rows, :], x_v.at[rows, :], x_sem.at[half])

    def wq_copy(h):
        return pltpu.make_async_copy(wq_hbm.at[:, pl.ds(h * cw, cw)], wq_v.at[h], wq_sem.at[h])

    def wq0_part_copy(r):
        cols = pl.ds(r * DH, DH)
        return pltpu.make_async_copy(wq_hbm.at[:, cols], wq_v.at[0, :, cols], wq0_sem.at[r])

    def wo_copy(p):
        return pltpu.make_async_copy(wot_hbm.at[:, pl.ds(p * HP * cw, HP * cw)], wo_v.at[p], wo_sem.at[p])

    def kv_start(it):
        g, p = gp(it)
        slot = it & 1
        for which, src in enumerate((k_hbm, v_hbm)):
            pltpu.make_async_copy(src.at[pl.ds(g * GB, GB), pl.ds(p * HP, HP)], kv_v.at[slot, which],
                                  kv_sem.at[slot]).start()

    def kv0_start(b):
        for which, src in enumerate((k_hbm, v_hbm)):
            pltpu.make_async_copy(src.at[b, pl.ds(0, HP)], kv_v.at[0, which, b], kv_sem.at[0]).start()

    def kv_wait(it):
        slot = it & 1
        pltpu.make_async_copy(kv_v.at[slot], kv_v.at[slot], kv_sem.at[slot]).wait()

    def out_copy(g):
        return pltpu.make_async_copy(out_v, o_hbm.at[pl.ds(g * m, m), :], o_sem.at[0])

    def out_tile_copy(g, j):
        return pltpu.make_async_copy(out_v.at[pl.ds(j * 128, 128), :],
                                     o_hbm.at[pl.ds(g * m + j * 128, 128), :], o_sem.at[0])

    def qpiece(h, r, b0=0, b1=GB):
        q = jnp.dot(x_v[b0 * sq:b1 * sq, :], wq_v[h, :, r * DH:(r + 1) * DH],
                    preferred_element_type=jnp.float32)
        q = (q * (DH ** -0.5 * LOG2E)).astype(jnp.bfloat16)
        for b in range(b0, b1):
            q_s[h, b, r * sq:(r + 1) * sq, :] = q[(b - b0) * sq:(b - b0 + 1) * sq]

    def attention(it):
        _, p = gp(it)
        slot = it & 1

        def qk(hh, b):
            return jax.lax.dot_general(q_s[p * HP + hh, b], kv_v[slot, 0, b, hh], NT,
                                       preferred_element_type=jnp.float32)

        def pv(s, hh, b):
            mx = jnp.max(s, axis=-1, keepdims=True)
            e = jnp.exp2(s - mx)
            l = jnp.sum(e, axis=-1, keepdims=True)
            o = jnp.dot(e.astype(jnp.bfloat16), kv_v[slot, 1, b, hh], preferred_element_type=jnp.float32)
            o = (o * (1.0 / l)).astype(jnp.bfloat16)
            return jnp.concatenate([o[r * sq:(r + 1) * sq] for r in range(rep)], axis=1)

        rows = [[] for _ in range(HP)]

        def otile(hh, j):
            a = jnp.concatenate(rows[hh], axis=0)[j * 128:(j + 1) * 128]
            part = jax.lax.dot_general(
                wo_v[p, :, hh * cw:(hh + 1) * cw], a, NT, preferred_element_type=jnp.float32)
            old = acc[:, j * 128:(j + 1) * 128]
            if hh == 0:
                old = jnp.where(p == 0, 0.0, old)
            acc[:, j * 128:(j + 1) * 128] = old + part

        seq = [(hh, b) for hh in range(HP) for b in range(GB)]
        n = len(seq)
        pending = [(hh, j) for hh in range(HP) for j in range(ntile)]
        svals = [qk(*seq[i]) for i in range(DEPTH)]
        for i, (hh, b) in enumerate(seq):
            if i + DEPTH < n:
                svals.append(qk(*seq[i + DEPTH]))
            rows[hh].append(pv(svals[i], hh, b))
            while pending and pending[0][0] * GB + ((pending[0][1] + 1) * 128 - 1) // sq < i:
                otile(*pending.pop(0))
        while pending:
            otile(*pending.pop(0))

    def body(it, c):
        g, p = gp(it)

        @pl.when(it < npair)
        def _():
            wo_copy(it).wait()

        kv_wait(it)

        @pl.when(it + 1 < nit)
        def _():
            kv_start(it + 1)

        @pl.when(it + 1 < npair)
        def _():
            wo_copy(it + 1).start()

        @pl.when(jnp.logical_and(p == 1, g + 1 < ngroups))
        def _():
            x_copy(g + 1).start()

        attention(it)

        @pl.when(jnp.logical_and(p == npair - 1, g + 1 < ngroups))
        def _():
            x_copy(g + 1).wait()

            @pl.when(g > 0)
            def _():
                out_copy(g - 1).wait()
            out_v[...] = acc[...].T.astype(out_v.dtype)
            out_copy(g).start()
            for h in range(hkv):
                for r in range(rep):
                    qpiece(h, r)
        return c

    x0_half_copy(0).start()
    wq0_part_copy(0).start()
    x0_half_copy(1).start()
    for r in range(1, rep):
        wq0_part_copy(r).start()
    wq_copy(1).start()
    x0_half_copy(0).wait()
    wq0_part_copy(0).wait()
    wq_copy(2).start()
    wq_copy(3).start()
    qpiece(0, 0, 0, GB // 2)
    x0_half_copy(1).wait()
    kv0_start(0)
    kv0_start(1)
    qpiece(0, 0, GB // 2, GB)
    for r in range(1, rep):
        wq0_part_copy(r).wait()
    wq_copy(1).wait()
    wq_copy(4).start()
    wq_copy(5).start()
    kv0_start(2)
    kv0_start(3)
    for r in range(1, rep):
        qpiece(0, r)
    for r in range(rep):
        qpiece(1, r)

    def pro_body(j, c):
        h = 2 * j
        wq_copy(h).wait()
        wq_copy(h + 1).wait()

        @pl.when(j == 1)
        def _():
            wq_copy(6).start()
            wq_copy(7).start()

        @pl.when(j < 3)
        def _():
            kv0_start(2 * j + 2)
            kv0_start(2 * j + 3)

        @pl.when(j == 2)
        def _():
            wo_copy(0).start()

        for hh in range(2):
            for r in range(rep):
                qpiece(h + hh, r)
        return c

    jax.lax.fori_loop(1, hkv // 2, pro_body, 0)

    jax.lax.fori_loop(0, nit, body, 0)

    gl = ngroups - 1
    if ngroups > 1:
        out_copy(gl - 1).wait()
    for j in range(ntile):
        out_v[j * 128:(j + 1) * 128, :] = acc[:, j * 128:(j + 1) * 128].T.astype(out_v.dtype)
        out_tile_copy(gl, j).start()
    out_copy(gl).wait()


@jax.jit
def pallas_standalone__gqa_block_cached__near_ridge_kernel(x, k_cache, v_cache, wq, wo):
    B, Sq, D = x.shape
    _, Hkv, Sk, Dh = k_cache.shape
    rep = HQ // Hkv
    ngroups = B // GB
    m = GB * Sq
    cw = rep * Dh
    bf = jnp.bfloat16
    kern = functools.partial(_kernel, sq=Sq, hkv=Hkv, rep=rep, ngroups=ngroups)
    hbm = pl.BlockSpec(memory_space=pltpu.HBM)
    out = pl.pallas_call(
        kern,
        in_specs=[hbm] * 5,
        out_specs=hbm,
        out_shape=jax.ShapeDtypeStruct((B * Sq, D), x.dtype),
        scratch_shapes=[
            pltpu.VMEM((m, D), bf),
            pltpu.VMEM((Hkv, D, cw), bf),
            pltpu.VMEM((Hkv // HP, D, HP * cw), bf),
            pltpu.VMEM((2, 2, GB, HP, Sk, Dh), bf),
            pltpu.VMEM((Hkv, GB, rep * Sq, Dh), bf),
            pltpu.VMEM((D, m), jnp.float32),
            pltpu.VMEM((m, D), bf),
            pltpu.SemaphoreType.DMA((2,)),
            pltpu.SemaphoreType.DMA((Hkv,)),
            pltpu.SemaphoreType.DMA((rep,)),
            pltpu.SemaphoreType.DMA((Hkv // HP,)),
            pltpu.SemaphoreType.DMA((2,)),
            pltpu.SemaphoreType.DMA((1,)),
        ],
        compiler_params=pltpu.CompilerParams(
            vmem_limit_bytes=126 * 1024 * 1024,
            disable_bounds_checks=True,
        ),
    )(x.reshape(B * Sq, D), k_cache, v_cache, wq, wo.T)
    return out.reshape(B, Sq, D)
```
